```python
import os as _os
_os.environ.setdefault("JAX_PLATFORMS", "cpu")
import jax
import jax.numpy as jnp

def _softmax(x, axis=-1):
    return jax.nn.softmax(x, axis=axis)
def _gelu(x):
    return jax.nn.gelu(x, approximate=True)
def _silu(x):
    return jax.nn.silu(x)
def _sigmoid(x):
    return jax.nn.sigmoid(x)
def _layernorm(x, axis=-1, eps=1e-5):
    m = jnp.mean(x, axis=axis, keepdims=True)
    v = jnp.var(x, axis=axis, keepdims=True)
    return (x - m) / jnp.sqrt(v + eps)
def _scatter_add(tgt, idx, src, axis=0):
    return tgt.at[idx].add(src)
def _segment_sum(src, seg, n):
    return jax.ops.segment_sum(src, seg, n)
class _Rng:
    def __init__(self, key):
        self._k = key
    def _next(self):
        self._k, sub = jax.random.split(self._k)
        return sub
    def normal(self, shape):
        return jax.random.normal(self._next(), shape, dtype=jnp.bfloat16)
    def randint(self, lo, hi, shape):
        return jax.random.randint(self._next(), shape, lo, hi, dtype=jnp.int32)
    def uniform(self, shape, lo=0.0, hi=1.0):
        return jax.random.uniform(self._next(), shape, jnp.bfloat16, lo, hi)
    def permutation(self, n):
        return jax.random.permutation(self._next(), n)


kernel_name = 'sequential_preLN__sliding_block__dense_activation_relu__prompt'

def setup_inputs():
    _rng = _Rng(jax.random.key(int.from_bytes(__import__("os").urandom(4), "little")))
    _w = (lambda a: (lambda t: t.astype(jnp.bfloat16) if jnp.issubdtype(t.dtype, jnp.floating) else t)(jnp.asarray(a)))
    def _A_setup():
        B, S, D = 1, 2048, 640
        return {
            "x": _w((lambda *s: _rng.normal(s) * 0.05)(B, S, D)),
            "wqkv": _w((lambda *s: _rng.normal(s) * 0.05)(D, 3 * D)),
            "wo": _w((lambda *s: _rng.normal(s) * 0.05)(D, D)),
        }
    _A_in = _A_setup()

    def _B_setup():
        B, S, D, Dff = 1, 2048, 640, 1536
        return {
            "x": _w((lambda *s: _rng.normal(s) * 0.05)(B, S, D)),
            "w1": _w((lambda *s: _rng.normal(s) * 0.05)(D, Dff)),
            "w2": _w((lambda *s: _rng.normal(s) * 0.05)(Dff, D)),
        }
    _B_in = _B_setup()

    return {
        "A_x": _A_in["x"],
        "A_wqkv": _A_in["wqkv"],
        "A_wo": _A_in["wo"],
        "B_x": _B_in["x"],
        "B_w1": _B_in["w1"],
        "B_w2": _B_in["w2"],
    }

def reference(A_x, A_wqkv, A_wo, B_x, B_w1, B_w2):
    def _A_ref(x, wqkv, wo):
        B, S, D = x.shape
        H = 32; Dh = D // H; W = 256
        qkv = (lambda x, *d: x.transpose(*d))((x @ wqkv).reshape(B, S, 3, H, Dh), 2, 0, 3, 1, 4)
        q, k, v = qkv[0], qkv[1], qkv[2]
        scores = jnp.einsum("bhqd,bhkd->bhqk", q, k) * (Dh ** -0.5)
        idx = jnp.arange(S)
        mask = (idx[:, None] - idx[None, :] >= 0) & (idx[:, None] - idx[None, :] < W)
        scores = jnp.where(mask[None, None], scores, -1e9)
        p = _softmax(scores, axis=-1)
        o = jnp.einsum("bhqk,bhkd->bhqd", p, v)
        return (lambda x, *d: x.transpose(*d))(o, 0, 2, 1, 3).reshape(B, S, D) @ wo

    def _B_ref(x, w1, w2):
        h = jnp.einsum("bsd,df->bsf", x, w1)
        zero = jnp.zeros_like(h)
        h = jnp.maximum(h, zero)
        return jnp.einsum("bsf,fd->bsd", h, w2)

    x = A_x
    h = x + _A_ref(_layernorm(x, axis=-1), A_wqkv, A_wo)
    h2 = h + _B_ref(_layernorm(h, axis=-1), B_w1, B_w2)
    return h2
```

```python
import functools
import jax
import jax.numpy as jnp
import numpy as np
from jax import lax
from jax.experimental import pallas as pl
from jax.experimental.pallas import tpu as pltpu

H = 32
W = 256
EPS = 1e-5
NEG = -1e30
NT = (((1,), (1,)), ((), ()))
F32, BF16, U32, I32 = jnp.float32, jnp.bfloat16, jnp.uint32, jnp.int32


def _ln(x):
    mu = jnp.mean(x, axis=-1, keepdims=True)
    xc = x - mu
    var = jnp.mean(xc * xc, axis=-1, keepdims=True)
    return xc * lax.rsqrt(var + EPS)


def _b(x):
    return pltpu.bitcast(x, BF16)


def _pack2(a, b):
    return pltpu.pack_elementwise([a, b], packed_dtype=BF16)


def _pack(z):
    return jnp.concatenate([_pack2(z[r:r + 8], z[r + 8:r + 16]) for r in range(0, z.shape[0], 16)], axis=0)


def _dot(a, b):
    return jnp.dot(a, b, preferred_element_type=F32)


def make_kernel(blocks=(256,) * 8, depth=2, S=2048, D=640, DFF=1536, flags=None, lead=1, lag=3, vsplit=1, nblk_limit=None):
    DH = D // H
    NG = H // 4
    GW = 4 * DH
    ND, NF = D // 128, DFF // 128
    qscale = float(DH ** -0.5 * np.log2(np.e))
    if nblk_limit:
        blocks = blocks[:nblk_limit]
    starts = [sum(blocks[:i]) for i in range(len(blocks))]
    nblk = len(blocks)

    def kernel(x_hbm, wqkv_hbm, wo_hbm, w1_hbm, w2_hbm, o_hbm,
               x_v, wqkv_v, wo_v, w1_v, w2_v, o_v, sems, osems):
        cx = [pltpu.make_async_copy(x_hbm.at[pl.ds(starts[i], blocks[i])], x_v.at[pl.ds(starts[i], blocks[i])], sems.at[i]) for i in range(nblk)]
        cw = [pltpu.make_async_copy(h, v, sems.at[nblk + j]) for j, (h, v) in enumerate([(wqkv_hbm, wqkv_v), (wo_hbm, wo_v), (w1_hbm, w1_v), (w2_hbm, w2_v)])]
        co = [pltpu.make_async_copy(o_v.at[pl.ds(starts[i], blocks[i])], o_hbm.at[pl.ds(starts[i], blocks[i])], osems.at[i]) for i in range(nblk)]
        cx[0].start()
        cw[0].start()
        for c in cx[1:]:
            c.start()
        for c in cw[1:]:
            c.start()

        sub8 = lax.broadcasted_iota(I32, (8, 128), 0)
        lane8 = lax.broadcasted_iota(I32, (8, 128), 1)
        lane16 = lax.broadcasted_iota(I32, (16, 128), 1)
        row16 = lax.broadcasted_iota(I32, (16, 128), 0)
        lane32 = lax.broadcasted_iota(I32, (32, 128), 1)
        row32 = lax.broadcasted_iota(I32, (32, 128), 0)
        rq = lane32 & 31
        causal = row32 <= rq
        klo = ((row16 >> 3) << 4) + (row16 & 7)
        cmask = pltpu.bitcast(jnp.where(klo <= (lane16 & 31), 0x0000FFFF, 0) | jnp.where(klo + 8 <= (lane16 & 31), -65536, 0), U32)
        fmask = ~cmask
        m1 = (lane16 & 32) != 0
        m2 = (lane16 & 64) != 0
        zero16 = jnp.zeros((16, 128), U32)
        wvt = []

        qg, kg, vtg, otg = {}, {}, {}, {}

        def group_tile(t, G):
            m, off = divmod(G * GW, 128)
            if off + GW <= 128:
                return t[m]
            lane = lax.broadcasted_iota(I32, t[m].shape, 1)
            return jnp.where(lane >= off, t[m], t[m + 1])

        def qk_tasks(i, st):
            t0, T = starts[i], blocks[i]
            st['ln'] = _ln(x_v[t0:t0 + T, :].astype(F32))
            lnb = st['ln'].astype(BF16)
            cols = []
            for n in range(2 * ND):
                cols.append(_dot(lnb, wqkv_v[:, 128 * n:128 * (n + 1)]))
                yield 5 * T
            q = [pltpu.bitcast((c * qscale).astype(BF16), U32) for c in cols[:ND]]
            for G in range(NG):
                qq, kk = group_tile(q, G), group_tile(cols[ND:], G)
                for r in range(0, T, 32):
                    qg[G, t0 + r] = qq[r // 2:r // 2 + 16]
                    kg[G, t0 + r] = kk[r:r + 32]

        def v_tasks(i, st):
            t0, T = starts[i], blocks[i]
            lnp = _pack(st['ln'])
            M = D // vsplit
            for r in range(0, T, 128):
                parts = []
                for m in range(vsplit):
                    parts.append(lax.dot_general(wvt[0][m * M:(m + 1) * M], _b(lnp[r // 2:r // 2 + 64]), NT, preferred_element_type=F32))
                    yield 5 * M
                vt = jnp.concatenate(parts, axis=0)
                for p in range(H // 2):
                    a = 2 * DH * p
                    sh = vt[a + 16:a + 24]
                    vtg[2 * p, t0 + r] = jnp.concatenate([vt[a:a + 16], jnp.where(sub8 < 4, sh, 1.0)], axis=0)
                    vtg[2 * p + 1, t0 + r] = jnp.concatenate([jnp.where(sub8 >= 4, sh, 1.0), vt[a + 24:a + 40]], axis=0)

        def scores(qb, G):
            off = (G * GW) % 128
            hm = [((lane16 - off - DH * s) & 127) < DH for s in range(4)]
            out = []
            for g in range(4):
                q0 = qb + 32 * g
                R = jnp.concatenate([jnp.where(hm[(m - g) % 4], qg[G, q0], jnp.uint32(0)) for m in range(4)], axis=0)
                kk = jnp.concatenate([kg[G, r] for r in range(max(0, q0 - W), q0 + 32, 32)], axis=0)
                out.append(lax.dot_general(kk, _b(R), NT, preferred_element_type=F32))
            return out

        def softmax(ss):
            A = []
            for g, s in enumerate(ss):
                n = s.shape[0]
                full = n == W + 32
                tri = jnp.where(causal, s[n - 32:], s[:32] if full else NEG)
                lo = 32 if full else 0
                allv = jnp.concatenate([s[lo:n - 32], tri], axis=0) if n > 32 else tri
                p = _pack(jnp.exp2(allv - jnp.max(allv, axis=0, keepdims=True)))
                chunks = [None] * 12
                nm = allv.shape[0] // 32 - 1
                chunks[g + 8] = p[16 * nm:] & cmask
                if full:
                    chunks[g] = p[16 * nm:] & fmask
                for j in range(nm):
                    chunks[g + 8 - nm + j] = p[16 * j:16 * (j + 1)]
                A.append(chunks)

            def sel(m, a, c):
                if a is None and c is None:
                    return None
                return jnp.where(m, zero16 if a is None else a, zero16 if c is None else c)
            Bq = [[sel(m1, A[(t + 1) % 4][j], A[t][j]) for j in range(12)] for t in range(4)]
            Cq = [[sel(m2, Bq[(t + 2) % 4][j], Bq[t][j]) for j in range(12)] for t in range(4)]
            return [Cq[(-s_) % 4] for s_ in range(4)]

        def pv(qb, G, Ps):
            j0 = max(0, (W - qb) // 32)
            outs = [None] * 4
            for kt in range(j0 // 4, 3):
                for s_ in range(4):
                    P = _b(jnp.concatenate(Ps[s_][4 * kt:4 * kt + 4], axis=0))
                    d = _dot(vtg[4 * G + s_, qb - W + 128 * kt], P)
                    outs[s_] = d if outs[s_] is None else outs[s_] + d
            outs = [pltpu.roll(o, 128 - 32 * s_, 1) if s_ else o for s_, o in enumerate(outs)]
            for pr in range(2):
                e, od = outs[2 * pr], outs[2 * pr + 1]
                rec = 1.0 / jnp.where(sub8 >= 4, e[16:], od[:8])
                rrot = pltpu.roll(rec, 4, 0)
                ie = jnp.where(sub8 < 4, rrot, rec)
                io = jnp.where(sub8 < 4, rec, rrot)
                otg[2 * G + pr, qb] = jnp.concatenate(
                    [e[:8] * ie, e[8:16] * ie, jnp.where(sub8 < 4, e[16:], od[:8]) * rrot, od[8:16] * io, od[16:] * io], axis=0)

        def wo_tasks(i, st):
            t0, T = starts[i], blocks[i]
            o = jnp.concatenate([jnp.concatenate([otg[p, qb] for p in range(H // 2)], axis=0).T for qb in range(t0, t0 + T, 128)], axis=0).astype(BF16)
            cols = []
            for n in range(ND):
                cols.append(x_v[t0:t0 + T, 128 * n:128 * (n + 1)].astype(F32) + _dot(o, wo_v[:, 128 * n:128 * (n + 1)]))
                yield 5 * T
            st['h1'] = cols
            st['ln2'] = _ln(jnp.concatenate(cols, axis=1)).astype(BF16)

        def ffn_tasks(i, st):
            t0, T = starts[i], blocks[i]
            hid = []
            for n in range(NF):
                hid.append(jnp.maximum(_dot(st['ln2'], w1_v[:, 128 * n:128 * (n + 1)]), 0.0).astype(BF16))
                yield 5 * T
            hid = [jnp.concatenate(hid[c:c + 4], axis=1) for c in range(0, NF, 4)]
            acc = list(st['h1'])
            for c in range(NF // 4):
                for n in range(ND):
                    acc[n] = acc[n] + _dot(hid[c], w2_v[512 * c:512 * (c + 1), 128 * n:128 * (n + 1)])
                    if c == NF // 4 - 1:
                        o_v[t0:t0 + T, 128 * n:128 * (n + 1)] = acc[n].astype(BF16)
                    yield 4 * T
            co[i].start()

        sts = [dict() for _ in range(nblk)]

        def run(gen):
            for _ in gen:
                pass

        def wait(cs):
            for c in cs:
                c.wait()
            return
            yield

        cx[0].wait()
        cw[0].wait()
        wvt.append(wqkv_v[:, 2 * D:].astype(F32).T.astype(BF16))
        run(qk_tasks(0, sts[0]))
        run(v_tasks(0, sts[0]))
        pend = []
        for i in range(nblk):
            t0, T = starts[i], blocks[i]
            gens, cost = [], 0
            if i == 0:
                gens.append(wait(cx[1:]))
            if i + 1 < nblk:
                gens.append(qk_tasks(i + 1, sts[i + 1])); cost += 50 * blocks[i + 1]
            if i == 1:
                gens.append(wait(cw[1:]))
            if i >= 1:
                gens.append(wo_tasks(i - 1, sts[i - 1])); cost += 25 * blocks[i - 1]
            if i + 1 < nblk:
                gens.append(v_tasks(i + 1, sts[i + 1])); cost += 25 * blocks[i + 1]
            if i >= 1:
                gens.append(ffn_tasks(i - 1, sts[i - 1])); cost += 120 * blocks[i - 1]
            chain = (c for g in gens for c in g)
            its = [(qb, G) for qb in range(t0, t0 + T, 128) for G in range(NG)]
            done = 0
            skip = depth if i + 1 == nblk else 0
            for n, it in enumerate(its):
                pend.append((it, softmax(scores(*it))))
                if len(pend) > depth:
                    a, b = pend.pop(0)
                    pv(*a, b)
                while n >= skip and done < cost * (n + 1 - skip) / (len(its) - skip):
                    c = next(chain, None)
                    if c is None:
                        break
                    done += c
            run(chain)
        for a, b in pend:
            pv(*a, b)
        run(wo_tasks(nblk - 1, sts[-1]))
        run(ffn_tasks(nblk - 1, sts[-1]))
        for c in co:
            c.wait()

    def f(A_x, A_wqkv, A_wo, B_x, B_w1, B_w2):
        out = pl.pallas_call(
            kernel,
            in_specs=[pl.BlockSpec(memory_space=pl.ANY)] * 5,
            out_specs=pl.BlockSpec(memory_space=pl.ANY),
            out_shape=jax.ShapeDtypeStruct((S, D), A_x.dtype),
            scratch_shapes=[
                pltpu.VMEM((S, D), BF16), pltpu.VMEM((D, 3 * D), BF16), pltpu.VMEM((D, D), BF16),
                pltpu.VMEM((D, DFF), BF16), pltpu.VMEM((DFF, D), BF16), pltpu.VMEM((S, D), BF16),
                pltpu.SemaphoreType.DMA((len(blocks) + 4,)),
                pltpu.SemaphoreType.DMA((len(blocks),)),
            ],
            compiler_params=pltpu.CompilerParams(vmem_limit_bytes=100 * 2**20, flags=flags),
            name="fused",
        )(A_x.reshape(S, D), A_wqkv, A_wo, B_w1, B_w2)
        return out.reshape(A_x.shape)
    return f


@jax.jit
def pallas_sequential_preLN__sliding_block__dense_activation_relu__prompt_kernel(
    A_x: jax.Array,
    A_wqkv: jax.Array,
    A_wo: jax.Array,
    B_x: jax.Array,
    B_w1: jax.Array,
    B_w2: jax.Array,
):
    return make_kernel(**dict())(A_x, A_wqkv, A_wo, B_x, B_w1, B_w2)
```

```python
import collections

import jax
import jax.numpy as jnp
import numpy as np
from jax import lax
from jax.experimental import pallas as pl
from jax.experimental.pallas import tpu as pltpu

F32, BF16, U32, I32 = jnp.float32, jnp.bfloat16, jnp.uint32, jnp.int32
S, D, DFF, H, W = 2048, 640, 1536, 32, 256
EPS = 1e-5
MASKED = -1e30
T = 256
DH = D // H
NG, GW = H // 4, 4 * DH
ND = D // 128
HIGH = np.uint32(0xFFFF0000)
QSCALE = float(DH ** -0.5 * np.log2(np.e))

_OWN = {0: [((0, 1), (1, 1)), ((1, -1), (1, 0))],
        1: [((-1, 1), (0, 1)), ((1, 0), (1, 1))],
        2: [((0, 1), (0, 1)), ((1, 0), (1, 0))]}
_PAIR = {(0, 1): (((0, 1), (1, 0), (1, 0), (0, -1)), (0, -1, 0, -1, 0, 1, -1), (-1, 0, -1, 0, 1, 0, 1)),
         (0, 2): (((1, -1), (1, 0), (1, 1), (0, 1)), (-1, 0, 0, -1, 0, 1, -1), (0, -1, -1, 0, 1, 0, 1)),
         (1, 2): (((1, -1), (0, -1), (1, 1), (1, 0)), (0, -1, -1, 0, 1, 0, 1), (-1, 0, 0, -1, 0, 1, -1))}


def _plain(nk, nn, i, j, k):
    ek, en, e2 = np.eye(nk, dtype=int), np.eye(nn, dtype=int), np.eye(2, dtype=int)
    return [np.outer(ek[i], e2[k]), np.outer(ek[i], en[j]), np.outer(en[j], e2[k])]


def _checked(rounds):
    nk, nn = rounds[0][0][1].shape
    total = sum(np.einsum('ik,pq,jl->ikpqjl', *p) for r in rounds for p in r)
    assert np.array_equal(total, np.einsum('ip,qj,kl->ikpqjl', np.eye(nk), np.eye(nn), np.eye(2)))
    return rounds


def _scheme(nk, nn, nodes, plan):
    ek, en = np.eye(nk, dtype=int), np.eye(nn, dtype=int)
    new = lambda a, x: [a, np.zeros((nk, nn), int), x]
    w = {(u, v): np.outer(ek[p[0]], en[q[1]]) for u, p in enumerate(nodes) for v, q in enumerate(nodes)}
    pairs = sorted((it for r in plan for it in r if isinstance(it, tuple)), key=len)
    for u, v, z in (it for it in pairs if len(it) == 3):
        w[u, z], w[z, u] = w[u, z] - w[u, v], w[z, u] - w[v, u]
    node, made = {}, {}
    for u, (i, j, t) in enumerate(nodes):
        node[u] = (ek[i], en[j], t, [new(np.outer(ek[i], a), np.outer(en[j], x)) for a, x in _OWN[t]])
        for p in node[u][3]:
            p[1] += w[u, u]
    for it in pairs:
        p, q = node[it[0]], node[it[1] if len(it) == 2 else tuple(sorted(it[1:]))]
        wpq, wqp = w[it[0], it[1]], w[it[1], it[0]]
        if p[2] > q[2]:
            p, q, wpq, wqp = q, p, wqp, wpq
        g, cpq, cqp = _PAIR[p[2], q[2]]
        t = 3 - p[2] - q[2]
        made[it] = [new(np.outer(p[0] + q[0], a), np.outer(p[1] + q[1], x)) for a, x in _OWN[t]]
        node[tuple(sorted(it))] = (p[0] + q[0], p[1] + q[1], t, list(made[it]))
        made[it].append(new(np.outer(p[0], g[0]) + np.outer(q[0], g[1]), np.outer(p[1], g[2]) + np.outer(q[1], g[3])))
        for z, a, b in zip(p[3] + q[3] + made[it], cpq, cqp):
            z[1] += a * wpq + b * wqp
    left = [list(node[u][3]) for u in range(len(nodes))]
    expand = lambda it: [left[it].pop()] if isinstance(it, int) else made[it] if isinstance(it, tuple) else [it]
    rounds = [[p for it in r for p in expand(it)] for r in plan]
    return _checked([r[2:] + r[:2] for r in rounds])


def _schemes():
    five = [[(0, 1, 2), 0], [(3, 2, 1), 3], [(1, 2), 1], [(0, 2), 2], [(0, 3), 0],
            [(1, 3), 1], [(0, 4), 4], [(1, 4), 4], [(2, 4), 2], [(3, 4), 3]]
    ten = lambda o: [[(o + p, o + 5 + (p + s) % 5), o + p if s <= 2 else o + 5 + (p + s) % 5]
                     for p in range(5) for s in (1, 2, 3, 4)]
    two = lambda x: [[(10, 11), 10], [(12, 13), 12], [10, 11, 11, x[0]], [12, 13, 13, x[1]], x[2:]]
    return dict(
        qkv=_scheme(5, 15, [(n, 10 + n, n // 2) for n in range(5)] + [(n % 5, n, n // 5) for n in range(10)],
                    five + ten(5)),
        wo=_scheme(5, 5, [(n, n, n // 2) for n in range(5)], five),
        w1=_scheme(5, 12, [(n % 5, n, n // 5) for n in range(10)] + [(n, 10 + n % 2, n % 2) for n in range(4)],
                   two([_plain(5, 12, 4, j, k) for j in (11, 10) for k in (1, 0)]) + ten(0)),
        w2=_scheme(12, 5, [(n, n % 5, n // 5) for n in range(10)] + [(10 + n % 2, n, n % 2) for n in range(4)],
                   two([_plain(12, 5, i, 4, k) for i in (11, 10) for k in (1, 0)]) + ten(0)))


def _startup(cols):
    items = [[_plain(5, 15, i, j, k) for j in cols for k in range(2)] for i in range(5)]
    return [[it[r:r + 4] for r in range(0, len(it), 4)] for it in items]


_PLAN = _schemes()
_START = [_startup([*range(10, 15), *range(10)]), _startup(range(10, 15))]
_FIRST = [_checked(sum(_START[0], [])), _checked(sum(_START[1], []) + _PLAN['qkv'][10:])]

_STAGE = dict(acc=96 * T, score=16 * T, diff=16 * T, cen=8 * T, norm=32 * T, qk=56 * T, v=64 * T, att=24 * T,
              res=16 * T, hid=28 * T, qkv=76 * 64, wo=26 * 64, w1=60 * 64, w2=60 * 64, mix=200 * 64)


class _Lazy:
    def __init__(self, get):
        self.get = get


class _Slot(_Lazy):
    def __init__(self, ring, at, n, dtype):
        self.ring, self.at, self.n, self.dtype = ring, at, n, dtype

    def __getitem__(self, rows):
        a, b, _ = rows.indices(self.n)
        return _Slot(self.ring, self.at + a, b - a, self.dtype)

    def _start(self):
        assert self.ring.pos - self.at <= self.ring.size, "staging slot reused too early"
        return self.at % self.ring.size

    def get(self):
        v = self.ring.ref[pl.ds(self._start(), self.n), :]
        return v if self.dtype == F32 else pltpu.bitcast(v, self.dtype)

    def set(self, v, stride=None):
        self.ring.last = self._start()
        self.ring.ref[pl.ds(self.ring.last, v.shape[0], stride), :] = v


class _Ring:
    def __init__(self, ref):
        self.ref, self.size, self.pos, self.last = ref, ref.shape[0], 0, None

    def new(self, n, dtype=F32):
        if self.pos % self.size + n > self.size:
            self.pos += self.size - self.pos % self.size
        self.pos += n
        return _Slot(self, self.pos - n, n, dtype)

    def put(self, v):
        raw = v if v.dtype == F32 else pltpu.bitcast(v, F32)
        slot = self.new(raw.shape[0], v.dtype)
        slot.set(raw)
        return slot


def _get(v):
    return v.get() if isinstance(v, _Lazy) else v


def _cat(parts):
    return jnp.concatenate([_get(p) for p in parts], axis=0)


def _sum(terms):
    pos, neg, sign = [v for s, v in terms if s > 0], [v for s, v in terms if s < 0], 1
    if not pos:
        pos, neg, sign = neg, [], -1
    out = _get(pos[0])
    for v in pos[1:]:
        out = out + _get(v)
    for v in neg:
        out = out - _get(v)
    return sign, out


def _words(x):
    return pltpu.bitcast(x.astype(BF16), U32)


def _join(lo, hi):
    return (lo >> 16) | (hi & HIGH)


def _zero_after(v):
    return pltpu.bitcast(jnp.minimum(lax.shift_right_logical(pltpu.bitcast(v, I32), 1), 0), U32)


def _eights(x):
    x = x.reshape(x.shape[0] // 16, 2, 8, 128)
    return [x[:, k].reshape(-1, 128) for k in range(2)]


def _dot(a, b):
    return jnp.dot(a, b, preferred_element_type=F32)


def _drain(queue):
    while queue:
        queue.popleft()()


def _take(gen, n):
    for _ in range(n):
        yield next(gen)


def _skip(gen, n):
    for _ in range(n):
        next(gen, None)


def _call(fn):
    fn()
    yield from ()


def _kernel(x_hbm, wqkv_hbm, wo_hbm, w1_hbm, w2_hbm, o_hbm,
            x_v, wqkv_v, wo_v, w1_v, w2_v, o_v, zero_s, load_sems, store_sems, *stage_v, P):
    nblk = P['nblk']
    rows = lambda a, b: (x_hbm.at[pl.ds(a * T, (b - a) * T)], x_v.at[pl.ds(a * T, (b - a) * T)])
    part = lambda i: (wqkv_hbm.at[pl.ds(128 * i, 128)], wqkv_v.at[pl.ds(128 * i, 128)])
    pairs = [rows(0, 1), part(0), rows(1, 2), part(1), part(2), part(3), part(4), rows(2, 4),
             (wo_hbm, wo_v), (w1_hbm, w1_v), (w2_hbm, w2_v), rows(4, S // T)]
    loads = collections.deque(pltpu.make_async_copy(a, b, load_sems.at[n]) for n, (a, b) in enumerate(pairs))
    stores = [pltpu.make_async_copy(o_v.at[pl.ds(i * T, T)], o_hbm.at[pl.ds(i * T, T)], store_sems.at[i])
              for i in range(nblk)]
    for copy in loads:
        copy.start()

    zero_s[0] = 0
    anywhere = lambda row: pl.ds(pl.multiple_of(zero_s[0] + row, 8), 8)
    for ref in stage_v:
        ref[anywhere(0), :] = jnp.zeros((8, 128), F32)
    ring = {name: _Ring(ref) for name, ref in zip(_STAGE, stage_v)}

    small, norms, mixes = (collections.deque() for _ in range(3))
    count, fences, gate = [0], [], []

    def arrive(n):
        fences.clear()
        gate.clear()
        for _ in range(n):
            loads.popleft().wait()

    def between(n_norm=1, n_mix=1):
        before = {c: ring[c].last for c in ('norm', 'cen', 'mix', 'att', 'qk')}
        for queue, n in ((small, 1), (norms, n_norm), (mixes, n_mix)):
            for _ in range(min(n, len(queue))):
                queue.popleft()()
        for c, last in before.items():
            if ring[c].last != last:
                fences.append((count[0] + P['fdelay'], ring[c].ref[anywhere(ring[c].last), :]))

    def fenced(w):
        for due, v in fences:
            if due <= count[0]:
                w = _cat([w[:-8], w[-8:] | _zero_after(v)])
        fences[:] = [f for f in fences if f[0] > count[0]]
        return w

    def run(gen, *rates):
        for _ in gen:
            between(*rates)

    weight_ref, weights = dict(qkv=wqkv_v, wo=wo_v, w1=w1_v, w2=w2_v), {}

    def weight(name, beta):
        if np.count_nonzero(beta) == 1 and beta.sum() < 0:
            return -1, weight(name, -beta)[1]
        key = name, beta.tobytes()
        if key not in weights:
            terms = []
            for i, j in zip(*np.nonzero(beta)):
                one = np.zeros_like(beta)
                one[i, j] = 1
                staged = weights.get((name, one.tobytes()))
                terms.append((beta[i, j], staged[1].get() if staged else
                              _words(weight_ref[name][128 * i:128 * (i + 1), 128 * j:128 * (j + 1)])))
            if len(terms) == 1:
                weights[key] = 1, ring[name].put(terms[0][1])
            else:
                if gate:
                    terms = [(s, v | _cat([gate[0]] * 8)) for s, v in terms]
                (sign, lo), (_, hi) = (_sum([(s, pltpu.bitcast(half(v), F32)) for s, v in terms])
                                       for half in (lambda v: v << 16, lambda v: v & HIGH))
                weights[key] = sign, ring['mix'].put(_join(*(pltpu.bitcast(z, U32) + np.uint32(0x8000) for z in (lo, hi))))
        return weights[key]

    def prepare(name, rounds, arrived=None):
        for r in rounds:
            betas = [b for _, b, _ in r if (name, b.tobytes()) not in weights and
                     (arrived is None or np.count_nonzero(b) > 1 and np.nonzero(b)[0].max() < arrived)]
            if betas:
                mixes.append(lambda betas=betas: [weight(name, b) for b in betas])

    def matmul(name, rounds, tiles, start, done):
        chan = {(i, c): t for i, halves in enumerate(tiles) for c, t in zip(((1, 0), (0, 1)), halves)}
        uses = collections.Counter(alpha.tobytes() for r in rounds for alpha, _, _ in r)
        made = {}

        def operand(alpha):
            key = alpha.tobytes()
            if key not in made:
                terms = []
                for i in np.nonzero(alpha.any(axis=1))[0]:
                    c = tuple(int(v) for v in alpha[i])
                    s = 1 if c in ((1, 0), (0, 1), (1, -1)) else -1
                    c = (s * c[0], s * c[1])
                    if (i, c) not in chan:
                        chan[i, c] = ring['diff'].put(_get(tiles[i][0]) - _get(tiles[i][1]))
                    terms.append((s, chan[i, c]))
                s, v = _sum(terms)
                made[key] = s, v.astype(BF16) if uses[key] > 1 or name in P['b16'] else v
            return made[key]

        acc = [[None if a is None else (1, a) for a in pair] for pair in start]
        last = {j: t for t, r in enumerate(rounds) for _, _, g in r for j in np.nonzero(g)[0]}
        for t, r in enumerate(rounds):
            h = T // 2 * len(r) // 4
            r = r[P['rot']:] + r[:P['rot']]
            groups = {}
            for (sa, a), (sw, w), gamma in [(operand(a), weight(name, b), g) for a, b, g in r]:
                w = pltpu.bitcast(fenced(w.get()), BF16)
                p = _cat([_dot(a[s:s + h], w) for s in range(0, T // 2, h)])
                for k in range(2):
                    outs = tuple(np.nonzero(gamma[:, k])[0])
                    if outs:
                        groups.setdefault((k, outs), []).append((gamma[outs[0], k] * sa * sw, p))
            count[0] += 1
            if not gate:
                gate.append(_zero_after(p[:8]))
            groups = {key: _sum(v) for key, v in groups.items()}
            for j in sorted({j for _, outs in groups for j in outs}):
                for k in range(2):
                    terms = [v for (kk, outs), v in groups.items() if kk == k and j in outs]
                    if terms:
                        s, v = _sum(terms + ([acc[j][k]] if acc[j][k] else []))
                        acc[j][k] = s, v if last[j] == t else ring['acc'].put(v)
                if last[j] == t:
                    done(j, [_get(v) if s > 0 else -_get(v) for s, v in acc[j]])
            yield h

    blocks = [{} for _ in range(nblk)]

    def layernorm(rows_of, i, name):
        n, held, out = P['lnc'], {}, []

        def step(r):
            if r + n < T:
                x = rows_of(r + n, n)
                x = x - jnp.mean(x, axis=-1, keepdims=True)
                scale = lax.rsqrt(jnp.mean(x * x, axis=-1, keepdims=True) + EPS)
                held[r + n] = scale, [ring['cen'].put(x[:, c:c + 128]) for c in range(0, D, 128)]
            if r == 0:
                out.extend(ring['norm'].new(T) for _ in range(ND))
            if r >= 0:
                for tile, x in zip(out, held[r][1]):
                    tile[r:r + n].set(x.get() * held[r][0])
            if r + n == T:
                blocks[i][name] = [[tile[:T // 2], tile[T // 2:]] for tile in out]
        norms.extend(lambda r=r: step(r) for r in range(-n, T, n))

    def normalised(i, name):
        while name not in blocks[i]:
            norms.popleft()()
        return blocks[i][name]

    def norm_input(i):
        layernorm(lambda r, n: x_v[i * T + r:i * T + r + n, :].astype(F32), i, 'ln1')

    sub8 = lax.broadcasted_iota(I32, (8, 128), 0)
    q_of, k_of, v_of, o_of = {}, {}, {}, {}

    def project(i, rounds):
        got = {}

        def groups(base, out):
            for g in range(NG):
                m, lane = divmod(g * GW, 128)
                need = (base + m,) if lane + GW <= 128 else (base + m, base + m + 1)
                if (g, i) not in out and all(n in got for n in need):
                    out[g, i] = got[need[0]]
                    if len(need) == 2:
                        lanes = lax.broadcasted_iota(I32, (T // 2, 128), 1)
                        out[g, i] = ring['qk'].put(jnp.where(lanes >= lane, got[need[0]].get(), got[need[1]].get()))

        def values(j, t, z):
            order = ring['v'].new(128)
            for k, rows8 in enumerate(_eights(z)):
                order[k:].set(rows8, stride=2)
            got[j, t] = ring['v'].put(order.get().T)
            for h in range(0, H, 2):
                tiles = [(2 * ND + a // 128, t) for a in range(DH * h, DH * (h + 2), 8)]
                if (h, t) not in v_of and all(n in got for n in tiles):
                    v = [got[n][(DH * h + 8 * m) % 128:][:8] for m, n in enumerate(tiles)]
                    shared = v[2].get()
                    v_of[h, t] = v[:2] + [ring['v'].put(jnp.where(sub8 < 4, shared, 1.0))]
                    v_of[h + 1, t] = [ring['v'].put(jnp.where(sub8 >= 4, shared, 1.0))] + v[3:]

        def done(j, halves):
            if j >= 2 * ND:
                for k, z in enumerate(halves):
                    values(j, i * T + 128 * k, z)
            elif j >= ND:
                got[j] = ring['qk'].put(_words(_cat(halves)))
                small.append(lambda: groups(ND, k_of))
            else:
                got[j] = ring['qk'].put(_words(_cat(halves) * QSCALE))
                small.append(lambda: groups(0, q_of))
        yield from matmul('qkv', rounds, normalised(i, 'ln1'), [[None] * 2] * (3 * ND), done)

    def attention_out(i):
        if (ND - 1, (i + 1) * T - 128) not in o_of:
            _drain(small)
        res = blocks[i]['res'] = [None] * ND
        x = [[_Lazy(lambda j=j, t=t: x_v[t:t + 128, 128 * j:128 * (j + 1)].astype(F32)) for t in (i * T, i * T + 128)]
             for j in range(ND)]

        def done(j, halves):
            res[j] = [ring['res'].put(z) for z in halves]
        yield from matmul('wo', _PLAN['wo'], [[o_of[j, i * T], o_of[j, i * T + 128]] for j in range(ND)], x, done)
        layernorm(lambda r, n: jnp.concatenate([z[r // 128][r % 128:][:n].get() for z in res], axis=1), i, 'ln2')

    def ffn_in(i):
        hid = blocks[i]['hid'] = [None] * (DFF // 128)

        def done(j, halves):
            hid[j] = [ring['hid'].put(jnp.maximum(z, 0.0)) for z in halves]
        yield from matmul('w1', _PLAN['w1'], normalised(i, 'ln2'), [[None] * 2] * len(hid), done)

    def ffn_out(i):
        def done(j, halves):
            o_v[i * T:(i + 1) * T, 128 * j:128 * (j + 1)] = _cat(halves).astype(o_v.dtype)
        yield from matmul('w2', _PLAN['w2'], blocks[i]['hid'], blocks[i]['res'], done)
        stores[i].start()

    lane16, row16 = (lax.broadcasted_iota(I32, (16, 128), a) for a in (1, 0))
    causal = lax.broadcasted_iota(I32, (32, 128), 0) <= (lax.broadcasted_iota(I32, (32, 128), 1) & 31)
    low_key = ((row16 >> 3) << 4) + (row16 & 7)
    near = pltpu.bitcast(jnp.where(low_key <= (lane16 & 31), 0xFFFF, 0) |
                         jnp.where(low_key + 8 <= (lane16 & 31), -0x10000, 0), U32)
    far = ~near
    odd, upper, nothing = (lane16 & 32) != 0, (lane16 & 64) != 0, jnp.zeros((16, 128), U32)

    def scores(t, g, u, split):
        t += 32 * u
        if (g, t // T) not in k_of or (g, t // T) not in q_of:
            _drain(small)
        q = q_of[g, t // T][t % T // 2:][:16].get()
        q = _cat([jnp.where(((lane16 - g * GW - DH * ((m - u) % 4)) & 127) < DH, q, nothing) for m in range(4)])
        first = max(0, t - W)
        k = _cat([k_of[g, b][max(first - b * T, 0) // 2:min(t + 32 - b * T, T) // 2]
                  for b in range(first // T, t // T + 1)])
        q, k = pltpu.bitcast(q, BF16), pltpu.bitcast(k, BF16)
        n = k.shape[0] // split
        return _cat([lax.dot_general(k[r:r + n], q, (((1,), (1,)), ((), ())), preferred_element_type=F32)
                     for r in range(0, k.shape[0], n)])

    def softmax(s, u):
        full = s.shape[0] == W + 32
        edge = jnp.where(causal, s[-32:], s[:32] if full else MASKED)
        s = _cat([s[32 * full:-32], edge]) if s.shape[0] > 32 else edge
        top = jnp.max(s, axis=0, keepdims=True)
        p = _join(*_eights(pltpu.bitcast(jnp.exp2(ring['score'].put(s).get() - top), U32)))
        chunks = [None] * 12
        chunks[u + 9 - p.shape[0] // 16:u + 8] = [p[r:r + 16] for r in range(0, p.shape[0] - 16, 16)]
        chunks[u + 8] = p[-16:] & near
        if full:
            chunks[u] = p[-16:] & far
        return chunks

    def per_head(a):
        def pick(mask, x, y):
            if x is None and y is None:
                return None
            return jnp.where(mask, nothing if x is None else x, nothing if y is None else y)
        only = [u for u in range(4) if a[u] is not None]
        if len(only) == 1:
            return [pick(lane16 >> 5 == (h + only[0]) % 4, a[only[0]], None) for h in range(4)]
        a = [pick(odd, a[(u + 1) % 4], a[u]) for u in range(4)]
        return [pick(upper, a[(2 - h) % 4], a[-h % 4]) for h in range(4)]

    def weigh_values(t, g, probs):
        out = [None] * 4
        steps = [m for m in P['ktord'] if t + 128 * m >= W]
        for m in steps:
            p = [per_head([a[c] for a in probs]) for c in range(4 * m, 4 * m + 4)[::-1 if P['desc'] else 1]][::-1 if P['desc'] else 1]
            new = [_dot(_cat(v_of[4 * g + h, t - W + 128 * m]), pltpu.bitcast(_cat([c[h] for c in p]), BF16))
                   for h in range(4)]
            out = [z if o is None else o + z for o, z in zip(out, new)]
            if m != steps[-1]:
                yield
        out = [pltpu.roll(o, 128 - 32 * h, 1) if h else o for h, o in enumerate(out)]
        for h in (0, 2):
            a, b = out[h], out[h + 1]
            inv = 1.0 / jnp.where(sub8 >= 4, a[16:], b[:8])
            swapped = pltpu.roll(inv, 4, 0)
            ia, ib = jnp.where(sub8 < 4, swapped, inv), jnp.where(sub8 < 4, inv, swapped)
            o_of['pair', 4 * g + h, t] = ring['att'].put(_cat(
                [a[:8] * ia, a[8:16] * ia, jnp.where(sub8 < 4, a[16:], b[:8]) * swapped, b[8:16] * ib, b[16:] * ib]))

        def transpose(j):
            cuts = [128 * j, *(a for a in range(0, D, 40) if 128 * j < a < 128 * (j + 1)), 128 * (j + 1)]
            o_of[j, t] = ring['att'].put(_cat(
                [o_of['pair', a // 40 * 2, t][a % 40:][:b - a] for a, b in zip(cuts, cuts[1:])]).T)
        small.extend(lambda j=j: transpose(j) for j in range(GW * g // 128, GW * (g + 1) // 128))
        yield

    arrive(1)
    norm_input(0)
    _drain(norms)
    first = [project(i, _FIRST[i]) for i in range(2)]
    for i, (a, b) in enumerate(zip(*_START)):
        arrive(1)
        mixes.clear()
        if i >= P['pfrom']:
            prepare('qkv', _PLAN['qkv'][10:], i + 1)
        if i == 0:
            run(_take(first[0], P['early']))
            arrive(1)
            norm_input(1)
            run(_take(first[0], len(a) - P['early']), len(norms) // (len(a) - P['early']))
        else:
            run(_take(first[0], len(a)))
        run(_take(first[1], len(b) - 2 * (i + 1 < ND)))
        _skip(first[1], 2 * (i + 1 < ND))
    run(first[0])
    run(_take(first[1], P['x2at'] - 2))
    _skip(first[1], 2)
    arrive(1)
    norm_input(2)
    prepare('qkv', _PLAN['qkv'][:10])
    run(first[1], P['ln2rate'])

    waiting = []

    def rest_arrives(gen):
        waiting.append(None)
        yield from _take(gen, 2)
        arrive(len(loads))
        for name in ('wo', 'w1', 'w2'):
            prepare(name, _PLAN[name])
        waiting.pop()
        yield from _take(gen, 1)

    pending = iter(())
    for i in range(nblk + 1):
        jobs, names = [], []
        if i + 2 < nblk:
            jobs.append(project(i + 2, _PLAN['qkv']))
            names.append('qkv')
        if i >= 2:
            jobs.append(ffn_out(i - 2))
            names.append('w2')
        dense = [_take(jobs[0], P['hold'])]
        if i == 1:
            dense = [_take(jobs[0], P['w1']), rest_arrives(jobs[0]), _take(jobs[0], P['qlead'])]
        if i >= 1:
            dense += [attention_out(i - 1), jobs.pop(0)]
            names += ['wo', 'w1']
        if i + 3 < nblk:
            dense.append(_call(lambda: norm_input(i + 3)))
        dense += jobs + ([ffn_in(i - 1)] if i >= 1 else [])
        dense = (cycles for gen in dense for cycles in gen)
        if i == nblk:
            run(_take(dense, 1))
            for gen in (pending, dense, ffn_out(i - 1)):
                run(gen)
            break
        width = lambda t: 1 if t >= W else 4 >> (t // 128)
        work = [(t, range(g, g + width(t))) for t in range(i * T, (i + 1) * T, 128) for g in range(0, NG, width(t))]
        keys = lambda t, u: min(t + 32 * u, W) + 32
        rate = sum(len(r) for name in names for r in _PLAN[name]) * T // 8
        total = sum(len(gs) * keys(t, u) for t, gs in work for u in range(4))
        issued = scored = 0
        for t, gs in work:
            probs = [[None] * 4 for _ in gs]
            join = 2 if t >= W else 1
            for u in range(4):
                if u % join == 0:
                    tiles = [(p, v, scores(t, g, v, 4 // len(gs) // join)) for v in (P['pairs'][u // 2] if join == 2 else [u])
                             for p, g in zip(probs, gs)]
                    for p, v, s in tiles:
                        p[v] = softmax(s, v)
                _skip(pending, len(gs) * P['pvat'][u])
                scored += len(gs) * keys(t, u) * (P['share'][u] if join == 2 else 1)
                while issued * total < rate * scored or waiting:
                    issued += next(dense)
                    if not waiting:
                        between()
            for _ in pending:
                pass
            pending = (None for gen in [weigh_values(t, g, p) for g, p in zip(gs, probs)] for _ in gen)
        run(dense)
    for copy in stores:
        copy.wait()


def make_kernel(nblk_limit=None, **kw):
    P = dict(nblk=nblk_limit or S // T, lnc=8, fdelay=6, early=5, x2at=6, ln2rate=3, hold=6, w1=11, qlead=13, pfrom=1, pvat=(0, 1, 2, 0), ktord=(1, 2, 0), rot=3, share=(.6, .6, 1.4, 1.4), pairs=((0, 1), (2, 3)), b16=(), desc=True)
    P.update(kw)

    def f(A_x, A_wqkv, A_wo, B_x, B_w1, B_w2):
        del B_x
        vmem = [pltpu.VMEM(s, BF16) for s in ((S, D), (D, 3 * D), (D, D), (D, DFF), (DFF, D), (S, D))]
        out = pl.pallas_call(
            lambda *refs: _kernel(*refs, P=P),
            in_specs=[pl.BlockSpec(memory_space=pl.ANY)] * 5,
            out_specs=pl.BlockSpec(memory_space=pl.ANY),
            out_shape=jax.ShapeDtypeStruct((S, D), A_x.dtype),
            scratch_shapes=vmem + [pltpu.SMEM((1,), I32), pltpu.SemaphoreType.DMA((12,)),
                                   pltpu.SemaphoreType.DMA((P['nblk'],))]
            + [pltpu.VMEM((n, 128), F32) for n in _STAGE.values()],
            compiler_params=pltpu.CompilerParams(vmem_limit_bytes=100 * 2**20),
            name="fused",
        )(A_x.reshape(S, D), A_wqkv, A_wo, B_w1, B_w2)
        return out.reshape(A_x.shape)
    return f


@jax.jit
def pallas_sequential_preLN__sliding_block__dense_activation_relu__prompt_kernel(
    A_x: jax.Array,
    A_wqkv: jax.Array,
    A_wo: jax.Array,
    B_x: jax.Array,
    B_w1: jax.Array,
    B_w2: jax.Array,
):
    return make_kernel(**dict())(A_x, A_wqkv, A_wo, B_x, B_w1, B_w2)
```

```python
import collections

import jax
import jax.numpy as jnp
import numpy as np
from jax import lax
from jax.experimental import pallas as pl
from jax.experimental.pallas import tpu as pltpu

F32, BF16, U32, I32 = jnp.float32, jnp.bfloat16, jnp.uint32, jnp.int32
S, D, DFF, H, W = 2048, 640, 1536, 32, 256
EPS = 1e-5
MASKED = -1e30
T = 256
BLOCKS = S // T
DH = D // H
NG, GW = H // 4, 4 * DH
ND = D // 128
HIGH = np.uint32(0xFFFF0000)
QSCALE = float(DH ** -0.5 * np.log2(np.e))

_OWN = {0: [((0, 1), (1, 1)), ((1, -1), (1, 0))],
        1: [((-1, 1), (0, 1)), ((1, 0), (1, 1))],
        2: [((0, 1), (0, 1)), ((1, 0), (1, 0))]}
_PAIR = {(0, 1): (((0, 1), (1, 0), (1, 0), (0, -1)), (0, -1, 0, -1, 0, 1, -1), (-1, 0, -1, 0, 1, 0, 1)),
         (0, 2): (((1, -1), (1, 0), (1, 1), (0, 1)), (-1, 0, 0, -1, 0, 1, -1), (0, -1, -1, 0, 1, 0, 1)),
         (1, 2): (((1, -1), (0, -1), (1, 1), (1, 0)), (0, -1, -1, 0, 1, 0, 1), (-1, 0, 0, -1, 0, 1, -1))}


def _plain(nk, nn, i, j, k):
    ek, en, e2 = np.eye(nk, dtype=int), np.eye(nn, dtype=int), np.eye(2, dtype=int)
    return [np.outer(ek[i], e2[k]), np.outer(ek[i], en[j]), np.outer(en[j], e2[k])]


def _checked(rounds):
    nk, nn = rounds[0][0][1].shape
    total = sum(np.einsum('ik,pq,jl->ikpqjl', *p) for r in rounds for p in r)
    assert np.array_equal(total, np.einsum('ip,qj,kl->ikpqjl', np.eye(nk), np.eye(nn), np.eye(2)))
    return rounds


def _scheme(nk, nn, nodes, plan):
    ek, en = np.eye(nk, dtype=int), np.eye(nn, dtype=int)
    new = lambda a, x: [a, np.zeros((nk, nn), int), x]
    w = {(u, v): np.outer(ek[p[0]], en[q[1]]) for u, p in enumerate(nodes) for v, q in enumerate(nodes)}
    pairs = sorted((it for r in plan for it in r if isinstance(it, tuple)), key=len)
    for u, v, z in (it for it in pairs if len(it) == 3):
        w[u, z], w[z, u] = w[u, z] - w[u, v], w[z, u] - w[v, u]
    node, made = {}, {}
    for u, (i, j, t) in enumerate(nodes):
        node[u] = (ek[i], en[j], t, [new(np.outer(ek[i], a), np.outer(en[j], x)) for a, x in _OWN[t]])
        for p in node[u][3]:
            p[1] += w[u, u]
    for it in pairs:
        p, q = node[it[0]], node[it[1] if len(it) == 2 else tuple(sorted(it[1:]))]
        wpq, wqp = w[it[0], it[1]], w[it[1], it[0]]
        if p[2] > q[2]:
            p, q, wpq, wqp = q, p, wqp, wpq
        g, cpq, cqp = _PAIR[p[2], q[2]]
        t = 3 - p[2] - q[2]
        made[it] = [new(np.outer(p[0] + q[0], a), np.outer(p[1] + q[1], x)) for a, x in _OWN[t]]
        node[tuple(sorted(it))] = (p[0] + q[0], p[1] + q[1], t, list(made[it]))
        made[it].append(new(np.outer(p[0], g[0]) + np.outer(q[0], g[1]), np.outer(p[1], g[2]) + np.outer(q[1], g[3])))
        for z, a, b in zip(p[3] + q[3] + made[it], cpq, cqp):
            z[1] += a * wpq + b * wqp
    left = [list(node[u][3]) for u in range(len(nodes))]
    expand = lambda it: [left[it].pop()] if isinstance(it, int) else made[it] if isinstance(it, tuple) else [it]
    rounds = [[p for it in r for p in expand(it)] for r in plan]
    return _checked([r[1:] + r[:1] if len(r) == 4 else r for r in rounds])


def _schemes():
    five = [[(0, 1, 2), 0], [(3, 2, 1), 3], [(1, 2), 1], [(0, 2), 2], [(0, 3), 0],
            [(1, 3), 1], [(0, 4), 4], [(1, 4), 4], [(2, 4), 2], [(3, 4), 3]]
    ten = lambda o: [[(o + p, o + 5 + (p + s) % 5), o + p if s <= 2 else o + 5 + (p + s) % 5]
                     for p in range(5) for s in (1, 2, 3, 4)]
    two = lambda x: [[(10, 11), 10], [(12, 13), 12], [10, 11, 11, x[0]], [12, 13, 13, x[1]], x[2:]]
    return dict(
        qkv=_scheme(5, 15, [(n, 10 + n, n // 2) for n in range(5)] + [(n % 5, n, n // 5) for n in range(10)],
                    five + ten(5)),
        wo=_scheme(5, 5, [(n, n, n // 2) for n in range(5)], five),
        w1=_scheme(5, 12, [(n % 5, n, n // 5) for n in range(10)] + [(n, 10 + n % 2, n % 2) for n in range(4)],
                   two([_plain(5, 12, 4, j, k) for j in (11, 10) for k in (1, 0)]) + ten(0)),
        w2=_scheme(12, 5, [(n, n % 5, n // 5) for n in range(10)] + [(10 + n % 2, n, n % 2) for n in range(4)],
                   two([_plain(12, 5, i, 4, k) for i in (11, 10) for k in (1, 0)]) + ten(0)))


def _startup(cols):
    items = [[_plain(5, 15, i, j, k) for j in cols for k in range(2)] for i in range(5)]
    return [[it[r:r + 4] for r in range(0, len(it), 4)] for it in items]


_PLAN = _schemes()
_START = [_startup([*range(10, 15), *range(10)]), _startup(range(10, 15))]
_FIRST = [_checked(sum(_START[0], [])), _checked(sum(_START[1], []) + _PLAN['qkv'][10:])]

_STAGE = dict(acc=96 * T, score=16 * T, diff=16 * T, cen=8 * T, norm=32 * T, qk=56 * T, v=64 * T, att=24 * T,
              res=16 * T, hid=28 * T, qkv=76 * 64, wo=26 * 64, w1=60 * 64, w2=60 * 64, mix=200 * 64)


class _Lazy:
    def __init__(self, get):
        self.get = get


class _Slot(_Lazy):
    def __init__(self, ring, at, n, dtype):
        self.ring, self.at, self.n, self.dtype = ring, at, n, dtype

    def __getitem__(self, rows):
        a, b, _ = rows.indices(self.n)
        return _Slot(self.ring, self.at + a, b - a, self.dtype)

    def _start(self):
        assert self.ring.pos - self.at <= self.ring.size, "staging slot reused too early"
        return self.at % self.ring.size

    def get(self):
        v = self.ring.ref[pl.ds(self._start(), self.n), :]
        return v if self.dtype == F32 else pltpu.bitcast(v, self.dtype)

    def set(self, v, stride=1):
        self.ring.last = self._start()
        self.ring.ref[pl.ds(self.ring.last, v.shape[0], stride), :] = v


class _Ring:
    def __init__(self, ref):
        self.ref, self.size, self.pos, self.last = ref, ref.shape[0] - 8, 0, None

    def new(self, n, dtype=F32):
        if self.pos % self.size + n > self.size:
            self.pos += self.size - self.pos % self.size
        self.pos += n
        return _Slot(self, self.pos - n, n, dtype)

    def put(self, v):
        raw = v if v.dtype == F32 else pltpu.bitcast(v, F32)
        slot = self.new(raw.shape[0], v.dtype)
        slot.set(raw)
        return slot


def _get(v):
    return v.get() if isinstance(v, _Lazy) else v


def _cat(parts):
    return jnp.concatenate([_get(p) for p in parts], axis=0)


def _sum(terms):
    pos, neg, sign = [v for s, v in terms if s > 0], [v for s, v in terms if s < 0], 1
    if not pos:
        pos, neg, sign = neg, [], -1
    out = _get(pos[0])
    for v in pos[1:]:
        out = out + _get(v)
    for v in neg:
        out = out - _get(v)
    return sign, out


def _words(x):
    return pltpu.bitcast(x.astype(BF16), U32)


def _join(lo, hi):
    return (lo >> 16) | (hi & HIGH)


def _zero_after(v):
    return pltpu.bitcast(jnp.minimum(lax.shift_right_logical(pltpu.bitcast(v, I32), 1), 0), U32)


def _eights(x):
    x = x.reshape(x.shape[0] // 16, 2, 8, 128)
    return [x[:, k].reshape(-1, 128) for k in range(2)]


def _dot(a, b):
    return jnp.dot(a, b, preferred_element_type=F32)


def _drain(queue):
    while queue:
        queue.popleft()()


def _take(gen, n):
    for _ in range(n):
        yield next(gen)


def _skip(gen, n):
    for _ in range(n):
        next(gen, None)


def _call(fn):
    fn()
    yield from ()


def _kernel(x_hbm, wqkv_hbm, wo_hbm, w1_hbm, w2_hbm, o_hbm,
            x_v, wqkv_v, wo_v, w1_v, w2_v, o_v, zero_s, load_sems, store_sems, *stage_v):
    rows = lambda a, b: (x_hbm.at[pl.ds(a * T, (b - a) * T)], x_v.at[pl.ds(a * T, (b - a) * T)])
    part = lambda i: (wqkv_hbm.at[pl.ds(128 * i, 128)], wqkv_v.at[pl.ds(128 * i, 128)])
    pairs = [rows(0, 1), part(0), rows(1, 2), part(1), part(2), part(3), part(4), rows(2, 4),
             (wo_hbm, wo_v), (w1_hbm, w1_v), (w2_hbm, w2_v), rows(4, BLOCKS)]
    loads = collections.deque(pltpu.make_async_copy(a, b, load_sems.at[n]) for n, (a, b) in enumerate(pairs))
    stores = []

    def store(*where):
        stores.append(pltpu.make_async_copy(o_v.at[where], o_hbm.at[where], store_sems.at[len(stores)]))
        stores[-1].start()

    for copy in loads:
        copy.start()

    zero_s[0] = 0
    anywhere = lambda row: pl.ds(pl.multiple_of(zero_s[0] + row, 8), 8)
    for ref in stage_v:
        ref[anywhere(0), :] = jnp.zeros((8, 128), F32)
    ring = {name: _Ring(ref) for name, ref in zip(_STAGE, stage_v)}

    small, norms, mixes = (collections.deque() for _ in range(3))
    count, fences, gate = [0], [], []

    def arrive(n):
        fences.clear()
        gate.clear()
        for _ in range(n):
            loads.popleft().wait()

    def between(n_norm=1):
        before = {c: ring[c].last for c in ('norm', 'cen', 'mix', 'att', 'qk')}
        for queue, n in ((small, 1), (norms, n_norm), (mixes, 1)):
            for _ in range(min(n, len(queue))):
                queue.popleft()()
        for c, last in before.items():
            if ring[c].last != last:
                fences.append((count[0] + 6, ring[c].ref[anywhere(ring[c].last), :]))

    def fenced(w):
        for due, v in fences:
            if due <= count[0]:
                w = _cat([w[:-8], w[-8:] | _zero_after(v)])
        fences[:] = [f for f in fences if f[0] > count[0]]
        return w

    def run(gen, n_norm=1):
        for _ in gen:
            between(n_norm)

    weight_ref, weights = dict(qkv=wqkv_v, wo=wo_v, w1=w1_v, w2=w2_v), {}

    def weight(name, beta):
        if np.count_nonzero(beta) == 1 and beta.sum() < 0:
            return -1, weight(name, -beta)[1]
        key = name, beta.tobytes()
        if key not in weights:
            terms = []
            for i, j in zip(*np.nonzero(beta)):
                one = np.zeros_like(beta)
                one[i, j] = 1
                staged = weights.get((name, one.tobytes()))
                terms.append((beta[i, j], staged[1].get() if staged else
                              _words(weight_ref[name][128 * i:128 * (i + 1), 128 * j:128 * (j + 1)])))
            if len(terms) == 1:
                weights[key] = 1, ring[name].put(terms[0][1])
            else:
                shift, mask = (_cat([gate[0] | c] * 8) if gate else c for c in (np.uint32(16), HIGH))
                (sign, lo), (_, hi) = (_sum([(s, pltpu.bitcast(half(v), F32)) for s, v in terms])
                                       for half in (lambda v: v << shift, lambda v: v & mask))
                weights[key] = sign, ring['mix'].put(_join(*(pltpu.bitcast(z, U32) + np.uint32(0x8000) for z in (lo, hi))))
        return weights[key]

    def prepare(name, rounds, arrived=None):
        for r in rounds:
            betas = [b for _, b, _ in r if (name, b.tobytes()) not in weights and
                     (arrived is None or np.count_nonzero(b) > 1 and np.nonzero(b)[0].max() < arrived)]
            if betas:
                mixes.append(lambda betas=betas: [weight(name, b) for b in betas])

    def matmul(name, rounds, tiles, start, done):
        chan = {(i, c): t for i, halves in enumerate(tiles) for c, t in zip(((1, 0), (0, 1)), halves)}
        uses = collections.Counter(alpha.tobytes() for r in rounds for alpha, _, _ in r)
        made = {}

        def operand(alpha):
            key = alpha.tobytes()
            if key not in made:
                terms = []
                for i in np.nonzero(alpha.any(axis=1))[0]:
                    c = tuple(int(v) for v in alpha[i])
                    s = 1 if c in ((1, 0), (0, 1), (1, -1)) else -1
                    c = (s * c[0], s * c[1])
                    if (i, c) not in chan:
                        chan[i, c] = ring['diff'].put(_get(tiles[i][0]) - _get(tiles[i][1]))
                    terms.append((s, chan[i, c]))
                s, v = _sum(terms)
                made[key] = s, v.astype(BF16) if uses[key] > 1 else v
            return made[key]

        acc = [[None if a is None else (1, a) for a in pair] for pair in start]
        last = {j: t for t, r in enumerate(rounds) for _, _, g in r for j in np.nonzero(g)[0]}
        for t, r in enumerate(rounds):
            h = T // 2 * len(r) // 4
            groups = {}
            for (sa, a), (sw, w), gamma in [(operand(a), weight(name, b), g) for a, b, g in r]:
                w = pltpu.bitcast(fenced(w.get()), BF16)
                p = _cat([_dot(a[s:s + h], w) for s in range(0, T // 2, h)])
                for k in range(2):
                    outs = tuple(np.nonzero(gamma[:, k])[0])
                    if outs:
                        groups.setdefault((k, outs), []).append((gamma[outs[0], k] * sa * sw, p))
            count[0] += 1
            if not gate:
                gate.append(_zero_after(p[:8]))
            groups = {key: _sum(v) for key, v in groups.items()}
            for j in sorted({j for _, outs in groups for j in outs}):
                for k in range(2):
                    terms = [v for (kk, outs), v in groups.items() if kk == k and j in outs]
                    if terms:
                        s, v = _sum(terms + ([acc[j][k]] if acc[j][k] else []))
                        acc[j][k] = s, v if last[j] == t else ring['acc'].put(v)
                if last[j] == t:
                    done(j, [_get(v) if s > 0 else -_get(v) for s, v in acc[j]])
            yield h

    blocks = [{} for _ in range(BLOCKS)]

    def layernorm(rows_of, i, name):
        n, held, out = 8, {}, []

        def step(r):
            if r + n < T:
                x = rows_of(r + n, n)
                x = x - jnp.mean(x, axis=-1, keepdims=True)
                scale = lax.rsqrt(jnp.mean(x * x, axis=-1, keepdims=True) + EPS)
                held[r + n] = scale, [ring['cen'].put(x[:, c:c + 128]) for c in range(0, D, 128)]
            if r == 0:
                out.extend(ring['norm'].new(T) for _ in range(ND))
            if r >= 0:
                for tile, x in zip(out, held[r][1]):
                    tile[r:r + n].set(x.get() * held[r][0])
            if r + n == T:
                blocks[i][name] = [[tile[:T // 2], tile[T // 2:]] for tile in out]
        norms.extend(lambda r=r: step(r) for r in range(-n, T, n))

    def normalised(i, name):
        while name not in blocks[i]:
            norms.popleft()()
        return blocks[i][name]

    def norm_input(i):
        layernorm(lambda r, n: x_v[i * T + r:i * T + r + n, :].astype(F32), i, 'ln1')

    sub8 = lax.broadcasted_iota(I32, (8, 128), 0)
    q_of, k_of, v_of, o_of = {}, {}, {}, {}

    def project(i, rounds):
        got = {}

        def groups(base, out):
            for g in range(NG):
                m, lane = divmod(g * GW, 128)
                need = (base + m,) if lane + GW <= 128 else (base + m, base + m + 1)
                if (g, i) not in out and all(n in got for n in need):
                    out[g, i] = got[need[0]]
                    if len(need) == 2:
                        lanes = lax.broadcasted_iota(I32, (T // 2, 128), 1)
                        out[g, i] = ring['qk'].put(jnp.where(lanes >= lane, got[need[0]].get(), got[need[1]].get()))

        def values(j, t, z):
            order = ring['v'].new(128)
            for k, rows8 in enumerate(_eights(z)):
                order[k:].set(rows8, stride=2)
            got[j, t] = ring['v'].put(order.get().T)
            for h in range(0, H, 2):
                tiles = [(2 * ND + a // 128, t) for a in range(DH * h, DH * (h + 2), 8)]
                if (h, t) not in v_of and all(n in got for n in tiles):
                    v = [got[n][(DH * h + 8 * m) % 128:][:8] for m, n in enumerate(tiles)]
                    shared = v[2].get()
                    v_of[h, t] = v[:2] + [ring['v'].put(jnp.where(sub8 < 4, shared, 1.0))]
                    v_of[h + 1, t] = [ring['v'].put(jnp.where(sub8 >= 4, shared, 1.0))] + v[3:]

        def done(j, halves):
            if j >= 2 * ND:
                for k, z in enumerate(halves):
                    values(j, i * T + 128 * k, z)
            elif j >= ND:
                got[j] = ring['qk'].put(_words(_cat(halves)))
                small.append(lambda: groups(ND, k_of))
            else:
                got[j] = ring['qk'].put(_words(_cat(halves) * QSCALE))
                small.append(lambda: groups(0, q_of))
        yield from matmul('qkv', rounds, normalised(i, 'ln1'), [[None] * 2] * (3 * ND), done)

    def attention_out(i):
        if (ND - 1, (i + 1) * T - 128) not in o_of:
            _drain(small)
        res = blocks[i]['res'] = [None] * ND
        x = [[_Lazy(lambda j=j, t=t: x_v[t:t + 128, 128 * j:128 * (j + 1)].astype(F32)) for t in (i * T, i * T + 128)]
             for j in range(ND)]

        def done(j, halves):
            res[j] = [ring['res'].put(z) for z in halves]
        yield from matmul('wo', _PLAN['wo'], [[o_of[j, i * T], o_of[j, i * T + 128]] for j in range(ND)], x, done)
        layernorm(lambda r, n: jnp.concatenate([z[r // 128][r % 128:][:n].get() for z in res], axis=1), i, 'ln2')

    def ffn_in(i):
        hid = blocks[i]['hid'] = [None] * (DFF // 128)

        def done(j, halves):
            hid[j] = [ring['hid'].put(jnp.maximum(z, 0.0)) for z in halves]
        yield from matmul('w1', _PLAN['w1'], normalised(i, 'ln2'), [[None] * 2] * len(hid), done)

    def ffn_out(i):
        def done(j, halves):
            o_v[i * T:(i + 1) * T, 128 * j:128 * (j + 1)] = _cat(halves).astype(o_v.dtype)
            if i + 1 == BLOCKS:
                store(pl.ds(i * T, T), pl.ds(128 * j, 128))
        yield from matmul('w2', _PLAN['w2'], blocks[i]['hid'], blocks[i]['res'], done)
        if i + 1 < BLOCKS:
            store(pl.ds(i * T, T))

    lane16, row16 = (lax.broadcasted_iota(I32, (16, 128), a) for a in (1, 0))
    causal = lax.broadcasted_iota(I32, (32, 128), 0) <= (lax.broadcasted_iota(I32, (32, 128), 1) & 31)
    low_key = ((row16 >> 3) << 4) + (row16 & 7)
    near = pltpu.bitcast(jnp.where(low_key <= (lane16 & 31), 0xFFFF, 0) |
                         jnp.where(low_key + 8 <= (lane16 & 31), -0x10000, 0), U32)
    far = ~near
    lane64 = lax.broadcasted_iota(I32, (64, 128), 1)
    odd, upper, nothing = (lane64 & 32) != 0, (lane64 & 64) != 0, jnp.zeros((16, 128), U32)
    head_lanes = [((lane16 - DH * h) & 127) < DH for h in range(H)]

    def scores(t, g, u, split):
        t += 32 * u
        if (g, t // T) not in k_of or (g, t // T) not in q_of:
            _drain(small)
        q = q_of[g, t // T][t % T // 2:][:16].get()
        q = _cat([lax.select(head_lanes[4 * g + (m - u) % 4], q, nothing) for m in range(4)])
        first = max(0, t - W)
        k = _cat([k_of[g, b][max(first - b * T, 0) // 2:min(t + 32 - b * T, T) // 2]
                  for b in range(first // T, t // T + 1)])
        q, k = pltpu.bitcast(q, BF16), pltpu.bitcast(k, BF16)
        n = k.shape[0] // split
        return _cat([lax.dot_general(k[r:r + n], q, (((1,), (1,)), ((), ())), preferred_element_type=F32)
                     for r in range(0, k.shape[0], n)])

    def softmax(s, u):
        full = s.shape[0] == W + 32
        edge = jnp.where(causal, s[-32:], s[:32] if full else MASKED)
        s = _cat([s[32 * full:-32], edge]) if s.shape[0] > 32 else edge
        top = jnp.max(s, axis=0, keepdims=True)
        p = _join(*_eights(pltpu.bitcast(jnp.exp2(ring['score'].put(s).get() - top), U32)))
        seen = [p[-16:] & far] * full + [p[:-16]] * (s.shape[0] > 32) + [p[-16:] & near]
        return _cat([nothing] * (u + 9 - full - s.shape[0] // 32) + seen + [nothing] * (3 - u))

    def weigh_values(t, g, probs):
        out = [None] * 4
        steps = [m for m in (1, 2, 0) if t + 128 * m >= W]
        for m in steps:
            p = [a[64 * m:64 * (m + 1)] for a in probs]
            p = [lax.select(odd, p[(u + 1) % 4], p[u]) for u in range(4)]
            p = [lax.select(upper, p[(2 - h) % 4], p[-h % 4]) for h in range(4)]
            new = [_dot(_cat(v_of[4 * g + h, t - W + 128 * m]), pltpu.bitcast(p[h], BF16)) for h in range(4)]
            out = [z if o is None else o + z for o, z in zip(out, new)]
            if m != steps[-1]:
                yield
        out = [pltpu.roll(o, 128 - 32 * h, 1) if h else o for h, o in enumerate(out)]
        for h in (0, 2):
            a, b = out[h], out[h + 1]
            inv = 1.0 / jnp.where(sub8 >= 4, a[16:], b[:8])
            swapped = pltpu.roll(inv, 4, 0)
            ia, ib = jnp.where(sub8 < 4, swapped, inv), jnp.where(sub8 < 4, inv, swapped)
            o_of['pair', 4 * g + h, t] = ring['att'].put(_cat(
                [a[:8] * ia, a[8:16] * ia, jnp.where(sub8 < 4, a[16:], b[:8]) * swapped, b[8:16] * ib, b[16:] * ib]))

        def transpose(j):
            cuts = [128 * j, *(a for a in range(0, D, 40) if 128 * j < a < 128 * (j + 1)), 128 * (j + 1)]
            o_of[j, t] = ring['att'].put(_cat(
                [o_of['pair', a // 40 * 2, t][a % 40:][:b - a] for a, b in zip(cuts, cuts[1:])]).T)
        small.extend(lambda j=j: transpose(j) for j in range(GW * g // 128, GW * (g + 1) // 128))
        yield

    arrive(1)
    norm_input(0)
    _drain(norms)
    first = [project(i, _FIRST[i]) for i in range(2)]
    for i, (a, b) in enumerate(zip(*_START)):
        arrive(1)
        mixes.clear()
        prepare('qkv', _PLAN['qkv'][10:], i + 1)
        if i == 0:
            run(_take(first[0], 5))
            arrive(1)
            norm_input(1)
            run(_take(first[0], len(a) - 5), len(norms) // (len(a) - 5))
        else:
            run(_take(first[0], len(a)))
        run(_take(first[1], len(b) - 2 * (i + 1 < ND)))
        _skip(first[1], 2 * (i + 1 < ND))
    run(first[0])
    run(_take(first[1], 8))
    _skip(first[1], 2)
    arrive(1)
    norm_input(2)
    prepare('qkv', _PLAN['qkv'][:10])
    run(first[1], 4)

    waiting = []

    def rest_arrives(gen):
        waiting.append(None)
        yield from _take(gen, 2)
        arrive(len(loads))
        for name in ('wo', 'w1', 'w2'):
            prepare(name, _PLAN[name])
        waiting.pop()
        yield from _take(gen, 1)

    pending = iter(())
    for i in range(BLOCKS + 1):
        jobs, names = [], []
        if i + 2 < BLOCKS:
            jobs.append(project(i + 2, _PLAN['qkv']))
            names.append('qkv')
        if i >= 2:
            jobs.append(ffn_out(i - 2))
            names.append('w2')
        dense = [_take(jobs[0], 7)]
        if i == 1:
            dense = [_take(jobs[0], 16), rest_arrives(jobs[0]), _take(jobs[0], 10)]
        if i >= 1:
            dense += [attention_out(i - 1), jobs.pop(0)]
            names += ['wo', 'w1']
        if i + 3 < BLOCKS:
            dense.append(_call(lambda: norm_input(i + 3)))
        dense += jobs + ([ffn_in(i - 1)] if i >= 1 else [])
        dense = (cycles for gen in dense for cycles in gen)
        if i == BLOCKS:
            run(_take(dense, 1))
            for gen in (pending, dense, ffn_out(i - 1)):
                run(gen)
            break
        width = lambda t: 1 if t >= W else 4 >> (t // 128)
        work = [(t, range(g, g + width(t))) for t in range(i * T, (i + 1) * T, 128) for g in range(0, NG, width(t))]
        keys = lambda t, u: min(t + 32 * u, W) + 32
        rate = sum(len(r) for name in names for r in _PLAN[name]) * T // 8
        total = sum(len(gs) * keys(t, u) for t, gs in work for u in range(4))
        issued = scored = 0
        for t, gs in work:
            probs = [[None] * 4 for _ in gs]
            join = 2 if t >= W else 1
            for u in range(4):
                if u % join == 0:
                    tiles = [(p, v, scores(t, g, v, 4 // len(gs) // join)) for v in range(u, u + join)
                             for p, g in zip(probs, gs)]
                    for p, v, s in tiles:
                        p[v] = softmax(s, v)
                _skip(pending, len(gs) * (0, 1, 2, 0)[u])
                scored += len(gs) * keys(t, u) * ((0.5, 1.5)[u // 2] if join == 2 else 1)
                while issued * total < rate * scored or waiting:
                    issued += next(dense)
                    if not waiting:
                        between()
            for _ in pending:
                pass
            pending = (None for gen in [weigh_values(t, g, p) for g, p in zip(gs, probs)] for _ in gen)
        run(dense)
    for copy in stores:
        copy.wait()


@jax.jit
def pallas_sequential_preLN__sliding_block__dense_activation_relu__prompt_kernel(
    A_x: jax.Array,
    A_wqkv: jax.Array,
    A_wo: jax.Array,
    B_x: jax.Array,
    B_w1: jax.Array,
    B_w2: jax.Array,
):
    del B_x
    operands = [pltpu.VMEM(s, BF16) for s in ((S, D), (D, 3 * D), (D, D), (D, DFF), (DFF, D), (S, D))]
    out = pl.pallas_call(
        _kernel,
        in_specs=[pl.BlockSpec(memory_space=pl.ANY)] * 5,
        out_specs=pl.BlockSpec(memory_space=pl.ANY),
        out_shape=jax.ShapeDtypeStruct((S, D), A_x.dtype),
        scratch_shapes=operands
        + [pltpu.SMEM((1,), I32), pltpu.SemaphoreType.DMA((12,)), pltpu.SemaphoreType.DMA((BLOCKS - 1 + ND,))]
        + [pltpu.VMEM((n + 8, 128), F32) for n in _STAGE.values()],
        compiler_params=pltpu.CompilerParams(vmem_limit_bytes=100 * 2**20),
        name="fused_block",
    )(A_x.reshape(S, D), A_wqkv, A_wo, B_w1, B_w2)
    return out.reshape(A_x.shape)
```
